```python
import os as _os
_os.environ.setdefault("JAX_PLATFORMS", "cpu")
import jax
import jax.numpy as jnp

def _softmax(x, axis=-1):
    return jax.nn.softmax(x, axis=axis)
def _gelu(x):
    return jax.nn.gelu(x, approximate=True)
def _silu(x):
    return jax.nn.silu(x)
def _sigmoid(x):
    return jax.nn.sigmoid(x)
def _layernorm(x, axis=-1, eps=1e-5):
    m = jnp.mean(x, axis=axis, keepdims=True)
    v = jnp.var(x, axis=axis, keepdims=True)
    return (x - m) / jnp.sqrt(v + eps)
def _scatter_add(tgt, idx, src, axis=0):
    return tgt.at[idx].add(src)
def _segment_sum(src, seg, n):
    return jax.ops.segment_sum(src, seg, n)
class _Rng:
    def __init__(self, key):
        self._k = key
    def _next(self):
        self._k, sub = jax.random.split(self._k)
        return sub
    def normal(self, shape):
        return jax.random.normal(self._next(), shape, dtype=jnp.bfloat16)
    def randint(self, lo, hi, shape):
        return jax.random.randint(self._next(), shape, lo, hi, dtype=jnp.int32)
    def uniform(self, shape, lo=0.0, hi=1.0):
        return jax.random.uniform(self._next(), shape, jnp.bfloat16, lo, hi)
    def permutation(self, n):
        return jax.random.permutation(self._next(), n)


kernel_name = 'sequential_preLN__sliding_block__dense_activation_gelu__prompt'

def setup_inputs():
    _rng = _Rng(jax.random.key(int.from_bytes(__import__("os").urandom(4), "little")))
    _w = (lambda a: (lambda t: t.astype(jnp.bfloat16) if jnp.issubdtype(t.dtype, jnp.floating) else t)(jnp.asarray(a)))
    def _A_setup():
        B, S, D = 1, 2048, 640
        return {
            "x": _w((lambda *s: _rng.normal(s) * 0.05)(B, S, D)),
            "wqkv": _w((lambda *s: _rng.normal(s) * 0.05)(D, 3 * D)),
            "wo": _w((lambda *s: _rng.normal(s) * 0.05)(D, D)),
        }
    _A_in = _A_setup()

    def _B_setup():
        B, S, D, F = 1, 2048, 640, 1536
        return {
            "x": _w((lambda *s: _rng.normal(s) * 0.05)(B, S, D)),
            "w1": _w((lambda *s: _rng.normal(s) * 0.8)(D, F) * (D ** -0.5)),
            "b1": _w((lambda *s: _rng.normal(s) * 0.8)(F) * 0.01),
            "w2": _w((lambda *s: _rng.normal(s) * 0.8)(F, D) * (F ** -0.5)),
            "b2": _w((lambda *s: _rng.normal(s) * 0.05)(D) * 0.01),
        }
    _B_in = _B_setup()

    return {
        "A_x": _A_in["x"],
        "A_wqkv": _A_in["wqkv"],
        "A_wo": _A_in["wo"],
        "B_x": _B_in["x"],
        "B_w1": _B_in["w1"],
        "B_b1": _B_in["b1"],
        "B_w2": _B_in["w2"],
        "B_b2": _B_in["b2"],
    }

def reference(A_x, A_wqkv, A_wo, B_x, B_w1, B_b1, B_w2, B_b2):
    def _A_ref(x, wqkv, wo):
        B, S, D = x.shape
        H = 32; Dh = D // H; W = 256
        qkv = (lambda x, *d: x.transpose(*d))((x @ wqkv).reshape(B, S, 3, H, Dh), 2, 0, 3, 1, 4)
        q, k, v = qkv[0], qkv[1], qkv[2]
        scores = jnp.einsum("bhqd,bhkd->bhqk", q, k) * (Dh ** -0.5)
        idx = jnp.arange(S)
        mask = (idx[:, None] - idx[None, :] >= 0) & (idx[:, None] - idx[None, :] < W)
        scores = jnp.where(mask[None, None], scores, -1e9)
        p = _softmax(scores, axis=-1)
        o = jnp.einsum("bhqk,bhkd->bhqd", p, v)
        return (lambda x, *d: x.transpose(*d))(o, 0, 2, 1, 3).reshape(B, S, D) @ wo

    def _B_ref(x, w1, b1, w2, b2):
        h = jnp.einsum("bsd,df->bsf", x, w1) + b1
        h = _gelu(h)
        return jnp.einsum("bsf,fd->bsd", h, w2) + b2

    x = A_x
    h = x + _A_ref(_layernorm(x, axis=-1), A_wqkv, A_wo)
    h2 = h + _B_ref(_layernorm(h, axis=-1), B_w1, B_b1, B_w2, B_b2)
    return h2
```

```python
import math
import jax
import jax.numpy as jnp
from jax import lax
import jax.experimental.pallas as pl
import jax.experimental.pallas.tpu as pltpu

S, D, F, H, DH, W = 2048, 640, 1536, 32, 20, 256
TB = 128
NB = S // TB
NT = D // 128
LOG2E = math.log2(math.e)
NEG = -1e9 * LOG2E
BF, F32, U32 = jnp.bfloat16, jnp.float32, jnp.uint32
NT_DIMS = (((1,), (1,)), ((), ()))

def _dot(a, b):
    return jnp.dot(a, b, preferred_element_type=F32)

def _ln(x):
    m = jnp.mean(x, axis=-1, keepdims=True)
    d = x - m
    v = jnp.mean(d * d, axis=-1, keepdims=True)
    return d * lax.rsqrt(v + 1e-5)

def _gelu(x):
    c = math.sqrt(2.0 / math.pi)
    t = jnp.tanh(x * (c + (c * 0.044715) * (x * x)))
    hx = 0.5 * x
    return hx + hx * t

def interleave(*gens):
    gens = list(gens)
    while gens:
        g = min(gens, key=lambda e: e[0])
        try:
            g[0] = next(g[1])
        except StopIteration:
            gens.remove(g)

def kernel(x_hbm, wqkv_hbm, wo_hbm, w1_hbm, b1_ref, w2_hbm, b2_ref, out_hbm,
           x_v, wqkv, wo, w1, w2, q_s, k_s, vt_s, ot_s, h_s, g_s, xn_s, o_s, hn_s, bias_s, b1_s, b2_s, out_v, sems, osem):
    XC = 4
    xr = S // XC
    x_cp = [pltpu.make_async_copy(x_hbm.at[pl.ds(c * xr, xr)], x_v.at[pl.ds(c * xr, xr)], sems.at[c]) for c in range(XC)]
    w_cp = [pltpu.make_async_copy(a, b, sems.at[XC + n]) for n, (a, b) in enumerate(
        [(wqkv_hbm, wqkv), (wo_hbm, wo), (w1_hbm, w1), (w2_hbm, w2)])]
    x_cp[0].start(); w_cp[0].start()
    for c in x_cp[1:] + w_cp[1:]:
        c.start()

    r = lax.broadcasted_iota(jnp.int32, (32, 128), 0)
    l = lax.broadcasted_iota(jnp.int32, (32, 128), 1)
    j, qi = l >> 5, l & 31
    for var in range(2):
        for m in range(3):
            left = (j < m) | ((j == m) & (r > qi))
            right = (j > m + 1) | ((j == m + 1) & (r <= qi))
            ok = (left | right) if var else right
            bias_s[var, 32 * m:32 * m + 32] = jnp.where(ok, 0.0, NEG)
        if var:
            bias_s[var, 96:128] = jnp.where((j < 3) | (r > qi), 0.0, NEG)
        else:
            bias_s[var, 96:128] = jnp.full((32, 128), NEG, F32)
        bias_s[var, 128:160] = jnp.where((j > 0) | (r <= qi), 0.0, NEG)
    k_s[:, 0:W // 2, :] = jnp.zeros((18, W // 2, 128), U32)
    vt_s[0:2] = jnp.zeros((2, D // 2, 128), U32)

    b1_s[...] = b1_ref[...].astype(F32).reshape(1, F)
    b2_s[...] = b2_ref[...].astype(F32).reshape(1, D)
    lane = lambda n: lax.broadcasted_iota(jnp.int32, (n, 128), 1)

    def qkv(i):
        st = {}
        def task(n):
            def f():
                if n == 0:
                    xn_s[...] = _ln(x_v[pl.ds(pl.multiple_of(i * TB, TB), TB)].astype(F32)).astype(BF)
                y = _dot(xn_s[...], wqkv[:, 128 * n:128 * n + 128])
                part, t = divmod(n, NT)
                if part == 2:
                    vt_s[i + 2, 64 * t:64 * t + 64] = pltpu.bitcast(y.astype(BF).T, U32)
                    return
                if part == 0:
                    y = y * (DH ** -0.5 * LOG2E)
                ref = (q_s, k_s)[part]
                rs = pl.ds(pl.multiple_of(i * (TB // 2) + part * (W // 2), TB // 2), TB // 2)
                y = pltpu.bitcast(y.astype(BF), U32)
                yr = pltpu.roll(y, 64, 1)
                ref[t, rs] = y
                ref[9 + t, rs] = yr
                if t:
                    hi = lane(TB // 2) >= 64
                    ref[NT + t - 1, rs] = jnp.where(hi, st[0], y)
                    ref[9 + NT + t - 1, rs] = jnp.where(hi, yr, st[1])
                st[0], st[1] = y, yr
            return f
        return [task(n) for n in range(3 * NT)]

    def attn(i):
        base = i * (TB // 2)
        var = jnp.where(i >= 2, 1, 0)
        mid_ok = i >= 1
        rows = lambda o, n: pl.ds(pl.multiple_of(base + o // 2, 16), n // 2)
        nt = lambda a, b: lax.dot_general(pltpu.bitcast(a, BF), pltpu.bitcast(b, BF), NT_DIMS, preferred_element_type=F32)
        st = {}
        def qk(g):
            def f():
                hs = range(4 * g, 4 * g + 4)
                off = {h: (DH * h) % 128 for h in hs}
                t = {h: (DH * h) // 128 + (NT if off[h] + DH > 128 else 0) for h in hs}
                ma = lambda h, n: ((lane(n) - off[h]) & 127) < DH
                mb = lambda h, n: ((lane(n) - off[h] - 64) & 127) < DH
                smid, sm = {}, {}
                getq = lambda h: jnp.where(ma(h, 64), q_s[t[h], rows(0, TB)], jnp.uint32(0))
                for h in hs:
                    q = getq(h)
                    qr = jnp.where(mb(h, 48), q_s[9 + t[h], rows(32, 96)], jnp.uint32(0))
                    sm[h] = [nt(jnp.where(ma(h, 16), k_s[t[h], rows(32 * m, 32)], k_s[9 + t[h], rows(288 + 32 * m, 32)]),
                                jnp.concatenate([q[:16 * (m + 1)], qr[16 * m:]], axis=0)) for m in range(3)]
                for h in hs:
                    smid[h] = nt(k_s[t[h], rows(96, 192)], getq(h))
                for h in hs:
                    edge = jnp.concatenate(sm[h] + [smid[h][0:32], smid[h][160:192]], axis=0) + bias_s[var]
                    mid = smid[h][32:160]
                    mx = jnp.maximum(jnp.max(edge.reshape(20, 8, 128), axis=0),
                                     jnp.where(mid_ok, jnp.max(mid.reshape(16, 8, 128), axis=0), NEG))
                    mx = jnp.max(mx, axis=0, keepdims=True)
                    pe = jnp.exp2(edge - mx)
                    pm = jnp.exp2(mid - jnp.where(mid_ok, mx, -NEG))
                    st[h] = jnp.concatenate(
                        [jnp.where(lane(32) < 32 * (m + 1), pe[32 * m:32 * m + 32], 0.0) for m in range(3)]
                        + [pe[96:128], pm, pe[128:160]]
                        + [jnp.where(lane(32) >= 32 * (m + 1), pe[32 * m:32 * m + 32], 0.0) for m in range(3)],
                        axis=0).astype(BF)
            return f
        def pv(g):
            def f():
                sub = lax.broadcasted_iota(jnp.int32, (8, 128), 0)
                res = []
                for h in range(4 * g, 4 * g + 4):
                    r0 = (DH * h) // 16 * 8
                    low = (DH * h) % 16 < 8
                    vts = []
                    for kt in range(3):
                        a, b = vt_s[i + kt, r0:r0 + 8], vt_s[i + kt, r0 + 8:r0 + 16]
                        if low:
                            b = jnp.where(sub >= 4, jnp.uint32(0x3F803F80), b)
                        else:
                            a = jnp.where(sub < 4, jnp.uint32(0x3F803F80), a)
                        vts.append(jnp.concatenate([a, b], axis=0))
                    o = _dot(pltpu.bitcast(jnp.concatenate(vts, axis=1), BF), st.pop(h))
                    den, num = (o[24:32], o[0:24]) if low else (o[0:8], o[8:32])
                    inv = 1.0 / den
                    res.append([num[8 * n:8 * n + 8] * inv for n in range(3)])
                a, b, c, d = res
                lo = sub < 4
                o = jnp.concatenate([a[0], a[1], jnp.where(lo, a[2], b[0]), b[1], b[2],
                                     c[0], c[1], jnp.where(lo, c[2], d[0]), d[1], d[2]], axis=0)
                ot_s[i & 1, 80 * g:80 * g + 80] = o.astype(BF)
            return f
        return [qk(g) for g in range(H // 4)], [pv(g) for g in range(H // 4)]

    def ffn(i):
        rs = pl.ds(pl.multiple_of(i * TB, TB), TB)
        def proj(t):
            def f():
                cs = slice(128 * t, 128 * t + 128)
                if t == 0:
                    o_s[...] = ot_s[i & 1].T
                h_s[:, cs] = x_v[rs, cs].astype(F32) + _dot(o_s[...], wo[:, cs])
                if t == NT - 1:
                    hn_s[...] = _ln(h_s[...]).astype(BF)
            return f
        def up(t):
            def f():
                cs = slice(128 * t, 128 * t + 128)
                g_s[:, cs] = _gelu(_dot(hn_s[...], w1[:, cs]) + b1_s[:, cs]).astype(BF)
            return f
        def down(t):
            def f():
                cs = slice(128 * t, 128 * t + 128)
                out_v[rs, cs] = (_dot(g_s[...], w2[:, cs]) + b2_s[:, cs] + h_s[:, cs]).astype(BF)
                if t == NT - 1:
                    pltpu.make_async_copy(out_v.at[rs], out_hbm.at[rs], osem).start()
            return f
        return [proj(t) for t in range(NT)], [up(t) for t in range(F // 128)], [down(t) for t in range(NT)]

    def run(tasks):
        for f in tasks:
            f()

    def with_attn(i, fill):
        qk, pv = attn(i)
        run(fill[0])
        for g in range(H // 4):
            qk[g]()
            run(fill[g + 1])
            pv[g]()

    w_cp[0].wait()
    x_cp[0].wait()
    lax.fori_loop(0, AHEAD, lambda i, c: (run(qkv(i)), c)[1], 0)
    a = qkv(AHEAD)
    with_attn(0, [[]] + [a[2 * g:2 * g + 2] for g in range(8)])
    for c in x_cp[1:] + w_cp[1:]:
        c.wait()
    def full(i, c):
        a = qkv(i + AHEAD)
        p, u, d = ffn(i - 1)
        with_attn(i, SCHED3(a, p, u, d))
        return c
    lax.fori_loop(1, NB - AHEAD, full, 0)
    def tail(i, c):
        p, u, d = ffn(i - 1)
        with_attn(i, SCHED2(p, u, d))
        return c
    lax.fori_loop(NB - AHEAD, NB, tail, 0)
    run(sum(ffn(NB - 1), []))
    pltpu.make_async_copy(out_v, out_hbm, osem).wait()

AHEAD = 3
SCHED3 = lambda a, p, u, d: [[], p + a[0:3], a[3:7], u[0:4] + a[7:11], u[4:8], u[8:12] + a[11:15], d[0:2], d[2:4], d[4:5]]
SCHED2 = lambda p, u, d: [[], p, [], u[0:4], u[4:8], u[8:12], d[0:2], d[2:4], d[4:5]]

@jax.jit
def pallas_sequential_preLN__sliding_block__dense_activation_gelu__prompt_kernel(
        A_x, A_wqkv, A_wo, B_x, B_w1, B_b1, B_w2, B_b2):
    any_ = pl.BlockSpec(memory_space=pl.ANY)
    vm = pl.BlockSpec(memory_space=pltpu.VMEM)
    out = pl.pallas_call(
        kernel,
        out_shape=jax.ShapeDtypeStruct((S, D), BF),
        in_specs=[any_, any_, any_, any_, vm, any_, vm],
        out_specs=any_,
        scratch_shapes=[
            pltpu.VMEM((S, D), BF), pltpu.VMEM((D, 3 * D), BF), pltpu.VMEM((D, D), BF),
            pltpu.VMEM((D, F), BF), pltpu.VMEM((F, D), BF),
            pltpu.VMEM((18, S // 2, 128), U32), pltpu.VMEM((18, (S + W) // 2, 128), U32),
            pltpu.VMEM((NB + 2, D // 2, 128), U32), pltpu.VMEM((2, D, TB), BF),
            pltpu.VMEM((TB, D), F32), pltpu.VMEM((TB, F), BF)] + [pltpu.VMEM((TB, D), BF)] * 3 + [ pltpu.VMEM((2, 160, 128), F32), pltpu.VMEM((1, F), F32), pltpu.VMEM((1, D), F32),
            pltpu.VMEM((S, D), BF),
            pltpu.SemaphoreType.DMA((8,)), pltpu.SemaphoreType.DMA,
        ],
        compiler_params=pltpu.CompilerParams(vmem_limit_bytes=100 * 2**20),
    )(A_x.reshape(S, D), A_wqkv, A_wo, B_w1, B_b1, B_w2, B_b2)
    return out.reshape(1, S, D)
```

```python
import math

import jax
import jax.numpy as jnp
from jax import lax
import jax.experimental.pallas as pl
import jax.experimental.pallas.tpu as pltpu

S, D, F, H, DH, W = 2048, 640, 1536, 32, 20, 256
TB = 128
NB = S // TB
NT = D // 128
NQ = 2 * NT - 1
C = 32
NE = TB // C - 1
AHEAD = 5
P, P0 = AHEAD + 1, 3
WA, WB = 2, 7
UNROLL2, UNROLL3 = 2, 2
LOG2E = math.log2(math.e)
NEG = -1e9 * LOG2E
BF, F32, U32 = jnp.bfloat16, jnp.float32, jnp.uint32

ORDER0 = "nanana"
ORDER1 = "amamamam" + "aam" * 4 + "aaav" * 8
ORDER2 = "pepepppeemeemuvvuuveeuevuvmvueueevuumvvueeuemvuvdvededemvdvdvedeemvdvvdedvdeedvvmddvvvdd"
ORDER3 = "pnpepepeemepaemvavavaeueauemvuvuuveueuemuvvuuvueueaemvavavaeaeaaemvavavaededemddvvvdddededemddvdvvdvvvdd"
ORDER4 = ("ppepeppemeeemuvvuuveueemvuvvueueeuvumvvueeuemvudvvededemvvvdeddeevmvdvedeemvvvvvv"
          "ddPPPdPdPdddUUUUUUUUDUUUUDDDDDDDDDDDDDD")


def _dot(a, b):
    return jnp.dot(a, b, preferred_element_type=F32)


def _pack(x):
    return pltpu.bitcast(x.astype(BF), U32)


def _bf(x):
    return pltpu.bitcast(x, BF)


def _dot_nt(a, b):
    return lax.dot_general(_bf(a), _bf(b), (((1,), (1,)), ((), ())), preferred_element_type=F32)


def _lane(n):
    return lax.broadcasted_iota(jnp.int32, (n, 128), 1)


def _layernorm(x):
    d = x - jnp.mean(x, axis=-1, keepdims=True)
    return d * lax.rsqrt(jnp.mean(d * d, axis=-1, keepdims=True) + 1e-5)


def _gelu(x):
    c = math.sqrt(2.0 / math.pi)
    t = jnp.tanh(x * (c + (c * 0.044715) * (x * x)))
    hx = 0.5 * x
    return hx + hx * t


def _run(order, tasks):
    its = {k: iter(v) for k, v in tasks.items()}
    for ch in order:
        next(its[ch])()
    assert all(next(it, None) is None for it in its.values())


def _kernel(x_hbm, wqkv_hbm, wo_hbm, w1_hbm, b1_hbm, w2_hbm, b2_hbm, out_hbm,
            x_v, wqkv, wo, w1, w2, q_s, k_s, vt_s, ot_s, h_s, g_s, xn_s, o_s, hn_s,
            s0_s, s1_s, bias_s, b1_v, b2_v, b1_s, b2_s, out_v, sems, osem):
    cp = pltpu.make_async_copy
    x_cp = [cp(x_hbm.at[a * TB:b * TB], x_v.at[a * TB:b * TB], sems.at[n])
            for n, (a, b) in enumerate([(0, P0), (P0, P), (P, NB)])]
    w_cp = [cp(wqkv_hbm.at[:, a * 128:b * 128], wqkv.at[:, a * 128:b * 128], sems.at[3 + n])
            for n, (a, b) in enumerate([(0, WA), (WA, NT), (NT, WB), (WB, 3 * NT)])]
    b_cp = [cp(b1_hbm, b1_v, sems.at[7]), cp(b2_hbm, b2_v, sems.at[8])]
    ffn_cp = [cp(a, b, sems.at[9 + n])
              for n, (a, b) in enumerate([(wo_hbm, wo), (w1_hbm, w1), (w2_hbm, w2)])]
    for c in [x_cp[0], w_cp[0], w_cp[1], x_cp[1], w_cp[2]]:
        c.start()

    r = lax.broadcasted_iota(jnp.int32, (TB, 128), 0)
    left, right = _lane(TB) < r, _lane(TB) >= r + C
    bias_s[0, 0:TB] = jnp.where(right, 0.0, NEG)
    bias_s[1, 0:TB] = jnp.where(left | right, 0.0, NEG)
    for var in range(2):
        bias_s[var, TB:TB + C] = jnp.where(left, NEG, 0.0)[0:C]
    k_s[0:NQ, (W - TB) // 2:W // 2, :] = jnp.zeros((NQ, TB // 2, 128), U32)
    vt_s[1] = jnp.zeros((D // 2, 128), U32)

    def norm_x(i, slot):
        xn_s[slot] = _pack(_layernorm(x_v[pl.ds(pl.multiple_of(i * TB, TB), TB)].astype(F32)))

    def qkv(i, slot):
        prev = {}

        def task(n):
            def f():
                y = _dot(_bf(xn_s[slot]), wqkv[:, 128 * n:128 * n + 128])
                part, t = divmod(n, NT)
                if part == 2:
                    vt_s[i + 2, 64 * t:64 * t + 64] = pltpu.bitcast(y.astype(BF).T, U32)
                    return
                if part == 0:
                    y = y * (DH ** -0.5 * LOG2E)
                ref = (q_s, k_s)[part]
                rs = pl.ds(pl.multiple_of(i * (TB // 2) + part * (W // 2), TB // 2), TB // 2)
                y = _pack(y)
                yr = pltpu.roll(y, 64, 1)
                ref[t, rs] = y
                ref[NQ + t, rs] = yr
                if t:
                    hi = _lane(TB // 2) >= 64
                    ref[NT + t - 1, rs] = jnp.where(hi, prev[part][0], y)
                    ref[NQ + NT + t - 1, rs] = jnp.where(hi, yr, prev[part][1])
                prev[part] = y, yr
            return f
        return [task(n) for n in range(3 * NT)]

    def attn(i, par):
        first = isinstance(i, int) and i == 0
        var = jnp.where(i >= 2, 1, 0)
        zero = i >> 8
        rows = lambda o, n: pl.ds(pl.multiple_of(i * (TB // 2) + o // 2, 8), n // 2)
        off = lambda h: (DH * h) % 128
        tile = lambda h: (DH * h) // 128 + (NT if off(h) + DH > 128 else 0)
        own = lambda h, n, rot=0: ((_lane(n) - off(h) - rot) & 127) < DH
        buf = lambda h: (s0_s, s1_s)[(h // 4) % 2]
        slot = lambda h: h % 4 + (h // 8 * 4 if first else 0)
        query = lambda h, o, n, rot=0: jnp.where(
            own(h, n // 2, rot), q_s[tile(h) + (NQ if rot else 0), rows(o, n)], jnp.uint32(0))
        top, acc = {}, {}

        def stash(h, r0, sc):
            buf(h)[slot(h), r0:r0 + sc.shape[0]] = sc
            mx = jnp.max(sc.reshape(-1, 8, 128), axis=0)
            top[h] = jnp.maximum(top[h], mx) if h in top else mx

        def probs(h, kt):
            ex = lambda r0, n: jnp.exp2(buf(h)[slot(h) + zero, r0:r0 + n] - top[h])
            if kt == 1 or first:
                return ex(TB, TB)
            if kt == 0:
                parts = [jnp.where(_lane(C) < C * (m + 1), ex(C * m, C), 0.0) for m in range(NE)]
                return jnp.concatenate(parts + [ex(TB - C, C)], axis=0)
            parts = [jnp.where(_lane(C) >= C * (m + 1), ex(C * m, C), 0.0) for m in range(NE)]
            return jnp.concatenate([ex(W, C)] + parts, axis=0)

        def edge(g, m):
            def f():
                n0 = C * (m + 1)
                for h in range(4 * g, 4 * g + 4):
                    t = tile(h)
                    q = jnp.concatenate([query(h, 0, n0), query(h, n0, TB - n0, 64)], axis=0)
                    k = jnp.where(own(h, C // 2), k_s[t, rows(C * m, C)], k_s[NQ + t, rows(W + n0, C)])
                    stash(h, C * m, _dot_nt(k, q) + bias_s[var, C * m:n0])
            return f

        def mid(g):
            def f():
                for h in range(4 * g, 4 * g + 4):
                    q = query(h, 0, TB)
                    if first:
                        causal = lax.broadcasted_iota(jnp.int32, (TB, TB), 0) <= _lane(TB)
                        stash(h, TB, jnp.where(causal, _dot_nt(k_s[tile(h), rows(W, TB)], q), NEG))
                    else:
                        sc = _dot_nt(k_s[tile(h), rows(TB - C, TB + 2 * C)], q)
                        stash(h, TB - C, sc[0:C] + bias_s[var, TB - C:TB])
                        stash(h, TB, sc[C:C + TB])
                        stash(h, W, sc[C + TB:] + bias_s[var, TB:TB + C])
                    top[h] = jnp.max(top[h], axis=0, keepdims=True)
            return f

        def pv(g, kt, final):
            def f():
                lo = lax.broadcasted_iota(jnp.int32, (8, 128), 0) < 4
                ones = jnp.uint32(0x3F803F80)
                res = []
                for h in range(4 * g, 4 * g + 4):
                    r0 = (DH * h) // 16 * 8
                    low = (DH * h) % 16 < 8
                    a, b = vt_s[i + kt, r0:r0 + 8], vt_s[i + kt, r0 + 8:r0 + 16]
                    a, b = (a, jnp.where(lo, b, ones)) if low else (jnp.where(lo, ones, a), b)
                    o = _dot(_bf(jnp.concatenate([a, b], axis=0)), probs(h, kt).astype(BF))
                    if h in acc:
                        o = o + acc.pop(h)
                    if not final:
                        acc[h] = o
                        continue
                    den, num = (o[24:32], o[0:24]) if low else (o[0:8], o[8:32])
                    inv = 1.0 / den
                    res.append([num[8 * n:8 * n + 8] * inv for n in range(3)])
                if final:
                    a, b, c, d = res
                    ot_s[40 * g:40 * g + 40] = _pack(jnp.concatenate(
                        [a[0], a[1], jnp.where(lo, a[2], b[0]), b[1], b[2],
                         c[0], c[1], jnp.where(lo, c[2], d[0]), d[1], d[2]], axis=0))
                    for t in range(80 * g // 128, 80 * (g + 1) // 128):
                        o_s[par, :, 128 * t:128 * t + 128] = pltpu.bitcast(_bf(ot_s[64 * t:64 * t + 64]).T, U32)
            return f

        groups = range(H // 4)
        if first:
            return dict(m=[mid(g) for g in groups], v=[pv(g, 2, True) for g in groups])
        return dict(e=[edge(g, m) for g in groups for m in range(NE)], m=[mid(g) for g in groups],
                    v=[pv(g, kt, kt == 1) for g in groups for kt in (0, 2, 1)])

    def ffn(i, par, slot, fine=False):
        rs = pl.ds(pl.multiple_of(i * TB, TB), TB)
        acc = {}

        def proj(t):
            def f():
                cs = slice(128 * t, 128 * t + 128)
                h_s[slot, :, cs] = x_v[rs, cs].astype(F32) + _dot(_bf(o_s[par]), wo[:, cs])
                if t == NT - 1:
                    hn_s[slot] = _pack(_layernorm(h_s[slot]))
            return f

        def up(t):
            def f():
                cs = slice(128 * t, 128 * t + 128)
                g_s[slot, :, cs] = _pack(_gelu(_dot(_bf(hn_s[slot]), w1[:, cs]) + b1_s[:, cs]))
            return f

        def down(t, c):
            def f():
                cs, ks = slice(128 * t, 128 * t + 128), slice(512 * c, 512 * c + 512)
                y = _dot(_bf(g_s[slot, :, ks]), w2[ks, cs])
                y = y + (acc.pop(t) if c else b2_s[:, cs] + h_s[slot, :, cs])
                if c < 2:
                    acc[t] = y
                    return
                out_v[rs, cs] = y.astype(BF)
                if fine:
                    cp(out_v.at[rs, cs], out_hbm.at[rs, cs], osem).start()
                elif t == NT - 1:
                    cp(out_v.at[rs], out_hbm.at[rs], osem).start()
            return f
        return dict(p=[proj(t) for t in range(NT)], u=[up(t) for t in range(F // 128)],
                    d=[down(t, c) for t in range(NT) for c in range(3)])

    def loop(lo, hi, unroll, body):
        def step(n, c):
            for u in range(unroll):
                i = lo + n * unroll + u
                body(i, (lo + u if unroll % 2 == 0 else i) & 1, u)
            return c
        lax.fori_loop(0, (hi - lo) // unroll, step, 0)

    def full(i, par, u):
        _run(ORDER3, dict(n=[lambda: norm_x(i + AHEAD, u)], a=qkv(i + AHEAD, u),
                          **ffn(i - 1, 1 - par, u), **attn(i, par)))

    def tail(i, par, u):
        _run(ORDER2, dict(**ffn(i - 1, 1 - par, u), **attn(i, par)))

    def last():
        f = ffn(NB - 1, 1, 1, True)
        _run(ORDER4, dict(P=f["p"], U=f["u"], D=f["d"], **ffn(NB - 2, 0, 0), **attn(NB - 1, 1)))

    blocks = [qkv(b, b) for b in range(P)]
    pick = lambda ns, bs: [blocks[b][n] for n in ns for b in bs]
    early, late = range(P0), range(P0, P)
    x_cp[0].wait()
    for b in early:
        norm_x(b, b)
    w_cp[0].wait()
    for c in [w_cp[3]] + b_cp:
        c.start()
    for f in pick(range(WA), early):
        f()
    w_cp[1].wait()
    for c in ffn_cp + [x_cp[2]]:
        c.start()
    for f in pick(range(WA, NT), early):
        f()
    x_cp[1].wait()
    w_cp[2].wait()
    todo = pick(range(NT, WB), early) + pick(range(WB), late)
    _run(ORDER0.ljust(len(todo) + len(late), "a"),
         dict(n=[lambda b=b: norm_x(b, b) for b in late], a=todo))
    for c in [w_cp[3]] + b_cp:
        c.wait()
    b1_s[...] = b1_v[...].astype(F32).reshape(1, F)
    b2_s[...] = b2_v[...].astype(F32).reshape(1, D)
    todo = pick(range(WB, 3 * NT), [0]) + pick(range(WB, 3 * NT), range(1, P))
    _run(ORDER1.ljust(len(todo) + H // 2, "a"), dict(a=todo, **attn(0, 0)))
    for c in ffn_cp + [x_cp[2]]:
        c.wait()

    loop(1, NB - AHEAD, UNROLL3, full)
    loop(NB - AHEAD, NB - 1, UNROLL2, tail)
    last()
    cp(out_v, out_hbm, osem).wait()


@jax.jit
def pallas_sequential_preLN__sliding_block__dense_activation_gelu__prompt_kernel(
    A_x: jax.Array,
    A_wqkv: jax.Array,
    A_wo: jax.Array,
    B_x: jax.Array,
    B_w1: jax.Array,
    B_b1: jax.Array,
    B_w2: jax.Array,
    B_b2: jax.Array,
):
    del B_x
    hbm = pl.BlockSpec(memory_space=pl.ANY)
    vmem = pltpu.VMEM
    out = pl.pallas_call(
        _kernel,
        out_shape=jax.ShapeDtypeStruct((S, D), BF),
        in_specs=[hbm] * 7,
        out_specs=hbm,
        scratch_shapes=[
            vmem((S, D), BF), vmem((D, 3 * D), BF), vmem((D, D), BF), vmem((D, F), BF), vmem((F, D), BF),
            vmem((2 * NQ, S // 2, 128), U32), vmem((2 * NQ, (S + W) // 2, 128), U32),
            vmem((NB + 2, D // 2, 128), U32), vmem((D // 2, TB), U32),
            vmem((2, TB, D), F32), vmem((2, TB // 2, F), U32),
            vmem((P, TB // 2, D), U32), vmem((2, TB // 2, D), U32), vmem((2, TB // 2, D), U32),
            vmem((H // 2, W + C, 128), F32), vmem((H // 2, W + C, 128), F32),
            vmem((2, TB + C, 128), F32),
            vmem((F,), BF), vmem((D,), BF), vmem((1, F), F32), vmem((1, D), F32),
            vmem((S, D), BF),
            pltpu.SemaphoreType.DMA((12,)), pltpu.SemaphoreType.DMA,
        ],
        compiler_params=pltpu.CompilerParams(vmem_limit_bytes=100 * 2**20),
    )(A_x.reshape(S, D), A_wqkv, A_wo, B_w1, B_b1, B_w2, B_b2)
    return out.reshape(1, S, D)
```

```python
import math

import jax
import jax.numpy as jnp
from jax import lax
import jax.experimental.pallas as pl
import jax.experimental.pallas.tpu as pltpu

S, D, F, H, DH, W = 2048, 640, 1536, 32, 20, 256
TB = 128
NB = S // TB
NT = D // 128
NQ = 2 * NT - 1
C = 32
NE = TB // C - 1
P, P0 = 4, 3
WA, WB = 2, 8
LOG2E = math.log2(math.e)
NEG = -1e30
BF, F32, U32 = jnp.bfloat16, jnp.float32, jnp.uint32

ORDER1 = "aaamaamavmaaavmvmavamavvamamvmvmavvavvmmavaavmvvmaavavmavavmvavvavaa"
ORDER3 = ("pnpepepeemepaemvavavaeueauemvuvuuveueuemuvvuuvueueaemvavavaeaeaaemvavavaededemddvvvdddeded"
          "emddvdvvdvvdvPdNPePePeemePAemvAvAvAeUeAUemvvUUUveUeUemUvvUUvUeUeAemvAvAvAeAeAAemvAvAvDAeDe"
          "DemDvvvDDDeDDeDemDDvvDvvvvDD")
ORDER2 = ("pepeppeepeemmuvvuuveeuevuvmvueueevuumvvueeuemvuvdvededemvdvdvedeemvdvvddevdeedvmvddvvvPePe"
          "ddPePPemeemUvvUUveeUevUvmvUeUeevUUvvUmeeUemvUvDveDeDemvvDDveDeevmvDvDeeDvDevvmDDDvvvDD")
ORDER4 = "pppppPPPPuPuuuuuuuuUuuUuUdUdUUdUddUdUddUdUddUddddDDDDDDDDDDDDDDD"


def _dot(a, b):
    return jnp.dot(a, b, preferred_element_type=F32)


def _pack(x):
    return pltpu.bitcast(x.astype(BF), U32)


def _bf(x):
    return pltpu.bitcast(x, BF)


def _dot_nt(a, b):
    return lax.dot_general(_bf(a), _bf(b), (((1,), (1,)), ((), ())), preferred_element_type=F32)


def _lane(n):
    return lax.broadcasted_iota(jnp.int32, (n, 128), 1)


def _layernorm(x):
    d = x - jnp.mean(x, axis=-1, keepdims=True)
    return d * lax.rsqrt(jnp.mean(d * d, axis=-1, keepdims=True) + 1e-5)


def _gelu(x):
    c = math.sqrt(2.0 / math.pi)
    t = jnp.tanh(x * (c + (c * 0.044715) * (x * x)))
    hx = 0.5 * x
    return hx + hx * t


def _run(order, tasks):
    its = {k: iter(v) for k, v in tasks.items()}
    for ch in order:
        next(its[ch])()
    assert all(next(it, None) is None for it in its.values())


def _kernel(x_hbm, wqkv_hbm, wo_hbm, w1_hbm, b1_hbm, w2_hbm, b2_hbm, out_hbm,
            x_v, wqkv, wo, w1, w2, q_s, k_s, vt_s, ot_s, h_s, g_s, xn_s, o_s, hn_s,
            s0_s, s1_s, bias_s, b1_v, b2_v, b1_s, b2_s, out_v, sems, xsem, osem):
    cp = pltpu.make_async_copy
    x_cp = [cp(x_hbm.at[a * TB:b * TB], x_v.at[a * TB:b * TB], sems.at[n])
            for n, (a, b) in enumerate([(0, P0), (P0, P)])]
    w_cp = [cp(wqkv_hbm.at[:, a * 128:b * 128], wqkv.at[:, a * 128:b * 128], sems.at[2 + n])
            for n, (a, b) in enumerate([(0, WA), (WA, NT), (NT, WB), (WB, 3 * NT)])]
    ffn_cp = [cp(a, b, sems.at[6 + n]) for n, (a, b) in enumerate(
        [(b1_hbm, b1_v), (b2_hbm, b2_v), (wo_hbm, wo), (w1_hbm, w1), (w2_hbm, w2)])]

    def pair_cp(j):
        rs = pl.ds(pl.multiple_of(2 * j * TB, 2 * TB), 2 * TB)
        return cp(x_hbm.at[rs], x_v.at[rs], xsem.at[j])

    for c in [x_cp[0], w_cp[0], w_cp[1], x_cp[1], w_cp[2], w_cp[3]] + ffn_cp:
        c.start()
    pair_cp(P // 2).start()

    r = lax.broadcasted_iota(jnp.int32, (TB, 128), 0)
    left, right = _lane(TB) < r, _lane(TB) >= r + C
    bias_s[0:TB] = jnp.where(left | right, 0.0, NEG)
    bias_s[TB:TB + C] = jnp.where(left, NEG, 0.0)[0:C]

    def norm_x(i, slot):
        xn_s[slot] = _pack(_layernorm(x_v[pl.ds(pl.multiple_of(i * TB, TB), TB)].astype(F32)))

    def qkv(i, slot):
        prev = {}

        def task(n):
            def f():
                y = _dot(_bf(xn_s[slot]), wqkv[:, 128 * n:128 * n + 128])
                part, t = divmod(n, NT)
                if part == 2:
                    vt_s[i + 2, 64 * t:64 * t + 64] = pltpu.bitcast(y.astype(BF).T, U32)
                    return
                if part == 0:
                    y = y * (DH ** -0.5 * LOG2E)
                ref = (q_s, k_s)[part]
                rs = pl.ds(pl.multiple_of(i * (TB // 2) + part * (W // 2), TB // 2), TB // 2)
                y = _pack(y)
                yr = pltpu.roll(y, 64, 1)
                ref[t, rs] = y
                ref[NQ + t, rs] = yr
                if t:
                    hi = _lane(TB // 2) >= 64
                    ref[NT + t - 1, rs] = jnp.where(hi, prev[part][0], y)
                    ref[NQ + NT + t - 1, rs] = jnp.where(hi, yr, prev[part][1])
                prev[part] = y, yr
            return f
        return [task(n) for n in range(3 * NT)]

    def attn(i, par):
        first = isinstance(i, int) and i < 2
        zero = i >> 8
        rows = lambda o, n: pl.ds(pl.multiple_of(i * (TB // 2) + o // 2, 8), n // 2)
        off = lambda h: (DH * h) % 128
        tile = lambda h: (DH * h) // 128 + (NT if off(h) + DH > 128 else 0)
        own = lambda h, n, rot=0: ((_lane(n) - off(h) - rot) & 127) < DH
        buf = lambda h: (s0_s, s1_s)[(h // 4) % 2]
        query = lambda h, o, n, rot=0: jnp.where(
            own(h, n // 2, rot), q_s[tile(h) + (NQ if rot else 0), rows(o, n)], jnp.uint32(0))
        top, acc = {}, {}

        def stash(h, r0, sc):
            buf(h)[h % 4, r0:r0 + sc.shape[0]] = sc
            mx = jnp.max(sc.reshape(-1, 8, 128), axis=0)
            top[h] = jnp.maximum(top[h], mx) if h in top else mx

        def probs(h, kt):
            ex = lambda r0, n: jnp.exp2(buf(h)[h % 4 + zero, r0:r0 + n] - top[h])
            if kt == 1 or first:
                return ex(kt * TB, TB)
            if kt == 0:
                parts = [jnp.where(_lane(C) < C * (m + 1), ex(C * m, C), 0.0) for m in range(NE)]
                return jnp.concatenate(parts + [ex(TB - C, C)], axis=0)
            parts = [jnp.where(_lane(C) >= C * (m + 1), ex(C * m, C), 0.0) for m in range(NE)]
            return jnp.concatenate([ex(W, C)] + parts, axis=0)

        def edge(g, m):
            def f():
                n0 = C * (m + 1)
                for h in range(4 * g, 4 * g + 4):
                    t = tile(h)
                    q = jnp.concatenate([query(h, 0, n0), query(h, n0, TB - n0, 64)], axis=0)
                    k = jnp.where(own(h, C // 2), k_s[t, rows(C * m, C)], k_s[NQ + t, rows(W + n0, C)])
                    stash(h, C * m, _dot_nt(k, q) + bias_s[C * m:n0])
            return f

        def mid(g):
            def f():
                for h in range(4 * g, 4 * g + 4):
                    q = query(h, 0, TB)
                    if first:
                        causal = lax.broadcasted_iota(jnp.int32, (TB, TB), 0) <= _lane(TB)
                        sc = _dot_nt(k_s[tile(h), rows(W - i * TB, TB + i * TB)], q)
                        if i:
                            stash(h, TB, sc[0:TB])
                        stash(h, W, jnp.where(causal, sc[i * TB:], NEG))
                    else:
                        sc = _dot_nt(k_s[tile(h), rows(TB - C, TB + 2 * C)], q)
                        stash(h, TB - C, sc[0:C] + bias_s[TB - C:TB])
                        stash(h, TB, sc[C:C + TB])
                        stash(h, W, sc[C + TB:] + bias_s[TB:TB + C])
                    top[h] = jnp.max(top[h], axis=0, keepdims=True)
            return f

        def pv(g, kt, final):
            def f():
                lo = lax.broadcasted_iota(jnp.int32, (8, 128), 0) < 4
                ones = jnp.uint32(0x3F803F80)
                res = []
                for h in range(4 * g, 4 * g + 4):
                    r0 = (DH * h) // 16 * 8
                    low = (DH * h) % 16 < 8
                    a, b = vt_s[i + kt, r0:r0 + 8], vt_s[i + kt, r0 + 8:r0 + 16]
                    a, b = (a, jnp.where(lo, b, ones)) if low else (jnp.where(lo, ones, a), b)
                    o = _dot(_bf(jnp.concatenate([a, b], axis=0)), probs(h, kt).astype(BF))
                    if h in acc:
                        o = o + acc.pop(h)
                    if not final:
                        acc[h] = o
                        continue
                    den, num = (o[24:32], o[0:24]) if low else (o[0:8], o[8:32])
                    inv = 1.0 / den
                    res.append([num[8 * n:8 * n + 8] * inv for n in range(3)])
                if final:
                    a, b, c, d = res
                    ot_s[40 * g:40 * g + 40] = _pack(jnp.concatenate(
                        [a[0], a[1], jnp.where(lo, a[2], b[0]), b[1], b[2],
                         c[0], c[1], jnp.where(lo, c[2], d[0]), d[1], d[2]], axis=0))
                    for t in range(80 * g // 128, 80 * (g + 1) // 128):
                        o_s[par, :, 128 * t:128 * t + 128] = pltpu.bitcast(_bf(ot_s[64 * t:64 * t + 64]).T, U32)
            return f

        groups = range(H // 4)
        if first:
            return dict(m=[mid(g) for g in groups], v=[pv(g, kt, kt == 2) for g in groups for kt in range(2 - i, 3)])
        return dict(e=[edge(g, m) for g in groups for m in range(NE)], m=[mid(g) for g in groups],
                    v=[pv(g, kt, kt == 1) for g in groups for kt in (0, 2, 1)])

    def ffn(i, par, slot, fine):
        rs = pl.ds(pl.multiple_of(i * TB, TB), TB)
        acc = {}

        def proj(t):
            def f():
                cs = slice(128 * t, 128 * t + 128)
                h_s[slot, :, cs] = x_v[rs, cs].astype(F32) + _dot(_bf(o_s[par]), wo[:, cs])
                if t == NT - 1:
                    hn_s[slot] = _pack(_layernorm(h_s[slot]))
            return f

        def up(t):
            def f():
                cs = slice(128 * t, 128 * t + 128)
                g_s[slot, :, cs] = _pack(_gelu(_dot(_bf(hn_s[slot]), w1[:, cs]) + b1_s[:, cs]))
            return f

        def down(t, c):
            def f():
                cs, ks = slice(128 * t, 128 * t + 128), slice(512 * c, 512 * c + 512)
                y = _dot(_bf(g_s[slot, :, ks]), w2[ks, cs])
                y = y + (acc.pop(t) if c else b2_s[:, cs] + h_s[slot, :, cs])
                if c < 2:
                    acc[t] = y
                    return
                out_v[rs, cs] = y.astype(BF)
                if fine:
                    cp(out_v.at[rs, cs], out_hbm.at[rs, cs], osem).start()
                elif t == NT - 1:
                    cp(out_v.at[rs], out_hbm.at[rs], osem).start()
            return f
        return dict(p=[proj(t) for t in range(NT)], u=[up(t) for t in range(F // 128)],
                    d=[down(t, c) for t in range(NT) for c in range(3)])

    def both(t, u, separate=True):
        if separate:
            return dict(t, **{k.upper(): v for k, v in u.items()})
        return {k: t.get(k, []) + u[k] for k in u}

    qkv_pair = lambda j: both(*(dict(n=[lambda b=b: norm_x(2 * j + b, b)], a=qkv(2 * j + b, b)) for b in range(2)))
    attn_pair = lambda j: both(*(attn(2 * j + b, b) for b in range(2)), separate=False)
    ffn_pair = lambda j, fine=False: both(*(ffn(2 * j + b, b, b, fine) for b in range(2)))

    def full(j, c):
        pair_cp(j + P // 2 - 1).wait()
        _run(ORDER3, dict(**qkv_pair(j + P // 2 - 1), **ffn_pair(j - 1), **attn_pair(j)))
        return c

    def tail(j, c):
        _run(ORDER2, dict(**ffn_pair(j - 1), **attn_pair(j)))
        return c

    blocks = [qkv(b, b) for b in range(P)]
    pick = lambda ns, bs: [blocks[b][n] for n in ns for b in bs]
    early, late = range(P0), range(P0, P)
    x_cp[0].wait()
    for b in early:
        norm_x(b, b)
    w_cp[0].wait()
    for f in pick(range(WA), early):
        f()
    w_cp[1].wait()
    for f in pick(range(WA, NT), early):
        f()
    x_cp[1].wait()
    w_cp[2].wait()
    for b in late:
        norm_x(b, b)
    for f in pick(range(NT, WB), early) + pick(range(WB), late):
        f()
    w_cp[3].wait()
    todo = pick(range(WB, 3 * NT), range(2)) + pick(range(WB, 3 * NT), range(2, P))
    _run(ORDER1, dict(a=todo, **attn_pair(0)))
    for c in ffn_cp:
        c.wait()
    for j in range(P // 2 + 1, NB // 2):
        pair_cp(j).start()
    b1_s[...] = b1_v[...].astype(F32).reshape(1, F)
    b2_s[...] = b2_v[...].astype(F32).reshape(1, D)

    split = (NB - P) // 2 + 1
    lax.fori_loop(1, split, full, 0)
    lax.fori_loop(split, NB // 2, tail, 0)
    _run(ORDER4, ffn_pair(NB // 2 - 1, True))
    cp(out_v, out_hbm, osem).wait()


@jax.jit
def pallas_sequential_preLN__sliding_block__dense_activation_gelu__prompt_kernel(
    A_x: jax.Array,
    A_wqkv: jax.Array,
    A_wo: jax.Array,
    B_x: jax.Array,
    B_w1: jax.Array,
    B_b1: jax.Array,
    B_w2: jax.Array,
    B_b2: jax.Array,
):
    del B_x
    hbm = pl.BlockSpec(memory_space=pl.ANY)
    vmem = pltpu.VMEM
    out = pl.pallas_call(
        _kernel,
        out_shape=jax.ShapeDtypeStruct((S, D), BF),
        in_specs=[hbm] * 7,
        out_specs=hbm,
        scratch_shapes=[
            vmem((S, D), BF), vmem((D, 3 * D), BF), vmem((D, D), BF), vmem((D, F), BF), vmem((F, D), BF),
            vmem((2 * NQ, S // 2, 128), U32), vmem((2 * NQ, (S + W) // 2, 128), U32),
            vmem((NB + 2, D // 2, 128), U32), vmem((D // 2, TB), U32),
            vmem((2, TB, D), F32), vmem((2, TB // 2, F), U32),
            vmem((P, TB // 2, D), U32), vmem((2, TB // 2, D), U32), vmem((2, TB // 2, D), U32),
            vmem((4, W + TB, 128), F32), vmem((4, W + TB, 128), F32),
            vmem((TB + C, 128), F32),
            vmem((F,), BF), vmem((D,), BF), vmem((1, F), F32), vmem((1, D), F32),
            vmem((S, D), BF),
            pltpu.SemaphoreType.DMA((11,)), pltpu.SemaphoreType.DMA((NB // 2,)), pltpu.SemaphoreType.DMA,
        ],
        compiler_params=pltpu.CompilerParams(vmem_limit_bytes=100 * 2**20),
    )(A_x.reshape(S, D), A_wqkv, A_wo, B_w1, B_b1, B_w2, B_b2)
    return out.reshape(1, S, D)
```
